```python
import os as _os
_os.environ.setdefault("JAX_PLATFORMS", "cpu")
import jax
import jax.numpy as jnp

def _softmax(x, axis=-1):
    return jax.nn.softmax(x, axis=axis)
def _gelu(x):
    return jax.nn.gelu(x, approximate=True)
def _silu(x):
    return jax.nn.silu(x)
def _sigmoid(x):
    return jax.nn.sigmoid(x)
def _layernorm(x, axis=-1, eps=1e-5):
    m = jnp.mean(x, axis=axis, keepdims=True)
    v = jnp.var(x, axis=axis, keepdims=True)
    return (x - m) / jnp.sqrt(v + eps)
def _scatter_add(tgt, idx, src, axis=0):
    return tgt.at[idx].add(src)
def _segment_sum(src, seg, n):
    return jax.ops.segment_sum(src, seg, n)
class _Rng:
    def __init__(self, key):
        self._k = key
    def _next(self):
        self._k, sub = jax.random.split(self._k)
        return sub
    def normal(self, shape):
        return jax.random.normal(self._next(), shape, dtype=jnp.bfloat16)
    def randint(self, lo, hi, shape):
        return jax.random.randint(self._next(), shape, lo, hi, dtype=jnp.int32)
    def uniform(self, shape, lo=0.0, hi=1.0):
        return jax.random.uniform(self._next(), shape, jnp.bfloat16, lo, hi)
    def permutation(self, n):
        return jax.random.permutation(self._next(), n)


kernel_name = 'standalone__linear_kernel_rfa__decode'

def setup_inputs():
    _rng = _Rng(jax.random.key(int.from_bytes(__import__("os").urandom(4), "little")))
    _w = (lambda a: (lambda t: t.astype(jnp.bfloat16) if jnp.issubdtype(t.dtype, jnp.floating) else t)(jnp.asarray(a)))
    B, H, Sq, Sk, D, M = 2, 16, 1, 16384, 256, 16
    return {
        "q": _w((lambda *s: _rng.normal(s) * 0.4)(B, H, Sq, D)),
        "k": _w((lambda *s: _rng.normal(s) * 1.6)(B, H, Sk, D)),
        "v": _w((lambda *s: _rng.normal(s) * 1.6)(B, H, Sk, D)),
        "omega": _w((lambda *s: _rng.normal(s) * 1.6)(M, D)),
    }

def reference(q, k, v, omega):
    d = q.shape[-1]
    m = omega.shape[0]
    scale = float(d) ** -0.25
    qs = q * scale
    ks = k * scale
    q_proj = jnp.einsum("bhsd,md->bhsm", qs, omega)
    k_proj = jnp.einsum("bhsd,md->bhsm", ks, omega)
    q_sq = 0.5 * jnp.einsum("bhsd,bhsd->bhs", qs, qs)[..., None]
    k_sq = 0.5 * jnp.einsum("bhsd,bhsd->bhs", ks, ks)[..., None]
    inv_sqrt_m = float(m) ** -0.5
    phi_q = jnp.exp(q_proj - q_sq) * inv_sqrt_m + 1e-6
    phi_k = jnp.exp(k_proj - k_sq) * inv_sqrt_m + 1e-6
    kv = jnp.einsum("bhsm,bhsd->bhmd", phi_k, v)
    z  = jnp.einsum("bhsm->bhm", phi_k)
    num = jnp.einsum("bhqm,bhmd->bhqd", phi_q, kv)
    den = jnp.einsum("bhqm,bhm->bhq", phi_q, z)[..., None] + 1e-6
    return num / den
```

```python
import jax
import jax.numpy as jnp
from jax import lax
import jax.experimental.pallas as pl
import jax.experimental.pallas.tpu as pltpu

BF=jnp.bfloat16; F32=jnp.float32
EPS = 9.98377799987793e-07
def _r(x): return x.astype(BF).astype(F32)

def chunk_compute(k, v, om_s, acc_kv, acc_z):
    T=k.shape[0]
    kp = lax.dot_general(om_s, k, (((1,),(1,)),((),())), preferred_element_type=F32)
    kf = k.astype(F32)
    sq = (kf[:, :128]*kf[:, :128] + kf[:,128:]*kf[:,128:]).astype(BF)
    ones = jnp.ones((16,128),BF)
    ks = lax.dot_general(ones, sq, (((1,),(1,)),((),())), preferred_element_type=F32)
    e = _r(_r(kp*0.25) - _r(ks)*(1.0/32))
    p = _r(_r(jnp.exp(e))*0.25 + EPS)
    kv = jnp.dot(p.astype(BF), v, preferred_element_type=F32)
    z = p[:, :128]
    for i in range(1,T//128):
        z = z + p[:, i*128:(i+1)*128]
    return acc_kv+kv, acc_z+z

def finalize(q, om, kv, z):
    qf=q.astype(F32); of=om.astype(F32)
    qp=_r(jnp.sum(qf*0.25*of,axis=1,keepdims=True))
    qsq=_r(jnp.sum(qf*qf,axis=1,keepdims=True))*(1.0/32)
    pq=_r(_r(jnp.exp(_r(qp-qsq)))*0.25+EPS)
    kv=_r(kv); z=_r(jnp.sum(z,axis=1,keepdims=True))
    num=_r(jnp.sum(pq*kv,axis=0,keepdims=True))
    den=_r(_r(jnp.sum(pq*z,axis=0,keepdims=True))+EPS)
    return (num/den).astype(BF)

def make(T=512,P=64,NB=8,SUB=None,start_first=True):
    n=T//P
    SUB=SUB or T
    def body(q_ref,om_ref,k_hbm,v_hbm,o_ref,kb,vb,qf_ref,of_ref,sem):
        R,D=k_hbm.shape; N=R//T
        G=q_ref.shape[0]; cph=N//G
        def st(i,slot):
            s=pl.multiple_of(i*T,T)
            for p in range(n):
                for a,(src,dst) in enumerate(((k_hbm,kb),(v_hbm,vb))):
                    pltpu.make_async_copy(src.at[pl.ds(s+p*P,P),:],dst.at[slot,pl.ds(p*P,P),:],sem.at[slot,a]).start(priority=a)
        for i in range(NB-1): st(i,i)
        qf_ref[...]=q_ref[...].astype(F32)
        om=om_ref[...]
        def head(g,_):
            def step(j,c):
                i=g*cph+j
                nxt=i+NB-1
                @pl.when(nxt<N)
                def _(): st(nxt,nxt%NB)
                slot=i%NB
                pltpu.make_async_copy(kb.at[slot],kb.at[slot],sem.at[slot,0]).wait()
                pltpu.make_async_copy(vb.at[slot],vb.at[slot],sem.at[slot,1]).wait()
                for u in range(T//SUB):
                    c=chunk_compute(kb[slot,pl.ds(u*SUB,SUB),:],vb[slot,pl.ds(u*SUB,SUB),:],om,*c)
                return c
            kv,z=lax.fori_loop(0,cph,step,(jnp.zeros((16,D),F32),jnp.zeros((16,128),F32)))
            of_ref[pl.ds(g,1),:]=finalize(qf_ref[pl.ds(g,1),:],om,kv,z).astype(F32)
            return 0
        lax.fori_loop(0,G,head,0)
        o_ref[...]=of_ref[...].astype(BF)
    def fn(q,k,v,om):
        B,H,S,D=k.shape; G=B*H
        vm=pl.BlockSpec(memory_space=pltpu.VMEM); hb=pl.BlockSpec(memory_space=pl.ANY)
        o=pl.pallas_call(body,in_specs=[vm,vm,hb,hb],out_specs=vm,
            out_shape=jax.ShapeDtypeStruct((G,D),BF),
            scratch_shapes=[pltpu.VMEM((NB,T,D),BF),pltpu.VMEM((NB,T,D),BF),pltpu.VMEM((G,D),F32),pltpu.VMEM((G,D),F32),pltpu.SemaphoreType.DMA((NB,2))],
            compiler_params=pltpu.CompilerParams(vmem_limit_bytes=64*2**20),
        )(q.reshape(G,D),om,k.reshape(G*S,D),v.reshape(G*S,D))
        return o.reshape(q.shape)
    return fn

_fn = make(512, 64, 8, 512)

@jax.jit
def pallas_standalone__linear_kernel_rfa__decode_kernel(q, k, v, omega):
    return _fn(q, k, v, omega)
```

```python
import functools

import jax
import jax.numpy as jnp
import numpy as np
from jax import lax
import jax.experimental.pallas as pl
import jax.experimental.pallas.tpu as pltpu

BF16 = jnp.bfloat16
F32 = jnp.float32
EPS = float(np.asarray(1e-6, dtype=BF16))

GROUP = 512
PIECE = 32
SLOTS = 5

_NT = (((1,), (1,)), ((), ()))


def _bf(x):
    return x.astype(BF16).astype(F32)


def _phi(proj, sumsq, scale, inv_sqrt_m):
    e = _bf(_bf(proj * scale) - 0.5 * _bf(sumsq * (scale * scale)))
    return _bf(_bf(_bf(jnp.exp(e)) * inv_sqrt_m) + EPS)


def _kernel(q_hbm, om_hbm, k_hbm, v_hbm, o_ref,
            k_buf, v_buf, q_buf, om_buf, q32, o32, kv_sem, small_sem,
            *, scale, inv_sqrt_m):
    rows, d = k_hbm.shape
    heads = q_buf.shape[0]
    m = om_buf.shape[0]
    n_groups = rows // GROUP
    groups_per_head = n_groups // heads

    def start_group(i, slot):
        base = pl.multiple_of(i * GROUP, GROUP)
        for p in range(GROUP // PIECE):
            for a, (src, dst) in enumerate(((k_hbm, k_buf), (v_hbm, v_buf))):
                pltpu.make_async_copy(
                    src.at[pl.ds(base + p * PIECE, PIECE), :],
                    dst.at[slot, pl.ds(p * PIECE, PIECE), :],
                    kv_sem.at[slot, a],
                ).start(priority=a)

    def wait_group(buf, slot, a):
        pltpu.make_async_copy(buf.at[slot], buf.at[slot], kv_sem.at[slot, a]).wait()

    start_group(0, 0)
    q_copy = pltpu.make_async_copy(q_hbm, q_buf, small_sem.at[0])
    om_copy = pltpu.make_async_copy(om_hbm, om_buf, small_sem.at[1])
    q_copy.start()
    om_copy.start()
    for i in range(1, SLOTS - 1):
        start_group(i, i)
    q_copy.wait()
    om_copy.wait()
    q32[...] = q_buf[...].astype(F32)
    omega = om_buf[...]

    def head_body(h, _):
        def group_body(j, carry):
            kv, z = carry
            i = h * groups_per_head + j
            nxt = i + SLOTS - 1

            @pl.when(nxt < n_groups)
            def _():
                start_group(nxt, nxt % SLOTS)

            slot = i % SLOTS
            wait_group(k_buf, slot, 0)
            k = k_buf[slot]
            proj = lax.dot_general(omega, k, _NT, preferred_element_type=F32)
            kf = k.astype(F32)
            sq = kf[:, :128] * kf[:, :128]
            for c in range(128, d, 128):
                sq = sq + kf[:, c:c + 128] * kf[:, c:c + 128]
            hi = sq.astype(BF16)
            lo = (sq - hi.astype(F32)).astype(BF16)
            sumsq = lax.dot_general(
                jnp.ones((m, 256), BF16), jnp.concatenate([hi, lo], axis=1),
                _NT, preferred_element_type=F32)
            phi_k = _phi(proj, sumsq, scale, inv_sqrt_m)
            for c in range(0, GROUP, 128):
                z = z + phi_k[:, c:c + 128]
            wait_group(v_buf, slot, 1)
            kv = kv + jnp.dot(phi_k.astype(BF16), v_buf[slot],
                              preferred_element_type=F32)
            return kv, z

        kv, z = lax.fori_loop(
            0, groups_per_head, group_body,
            (jnp.zeros((m, d), F32), jnp.zeros((m, 128), F32)))

        q = q32[pl.ds(h, 1), :]
        phi_q = _phi(jnp.sum(q * omega.astype(F32), axis=1, keepdims=True),
                     jnp.sum(q * q, axis=1, keepdims=True),
                     scale, inv_sqrt_m)
        z = _bf(jnp.sum(z, axis=1, keepdims=True))
        num = _bf(jnp.sum(phi_q * _bf(kv), axis=0, keepdims=True))
        den = _bf(_bf(jnp.sum(phi_q * z, axis=0, keepdims=True)) + EPS)
        o32[pl.ds(h, 1), :] = num / den
        return 0

    lax.fori_loop(0, heads, head_body, 0)
    o_ref[...] = o32[...].astype(o_ref.dtype)


@jax.jit
def pallas_standalone__linear_kernel_rfa__decode_kernel(
    q: jax.Array,
    k: jax.Array,
    v: jax.Array,
    omega: jax.Array,
):
    b, h, s, d = k.shape
    m = omega.shape[0]
    heads = b * h
    assert q.shape == (b, h, 1, d) and s % GROUP == 0 and d % 128 == 0
    assert heads * (s // GROUP) >= SLOTS - 1
    hbm = pl.BlockSpec(memory_space=pl.ANY)
    out = pl.pallas_call(
        functools.partial(_kernel, scale=float(d) ** -0.25,
                          inv_sqrt_m=float(m) ** -0.5),
        in_specs=[hbm, hbm, hbm, hbm],
        out_specs=pl.BlockSpec(memory_space=pltpu.VMEM),
        out_shape=jax.ShapeDtypeStruct((heads, d), q.dtype),
        scratch_shapes=[
            pltpu.VMEM((SLOTS, GROUP, d), k.dtype),
            pltpu.VMEM((SLOTS, GROUP, d), v.dtype),
            pltpu.VMEM((heads, d), q.dtype),
            pltpu.VMEM((m, d), omega.dtype),
            pltpu.VMEM((heads, d), F32),
            pltpu.VMEM((heads, d), F32),
            pltpu.SemaphoreType.DMA((SLOTS, 2)),
            pltpu.SemaphoreType.DMA((2,)),
        ],
        compiler_params=pltpu.CompilerParams(disable_bounds_checks=True),
    )(q.reshape(heads, d), omega, k.reshape(heads * s, d), v.reshape(heads * s, d))
    return out.reshape(q.shape)
```
